```python
import jax
import jax.numpy as jnp

def _softmax(x, axis=-1):
    return jax.nn.softmax(x, axis=axis)
def _gelu(x):
    return jax.nn.gelu(x, approximate=True)
def _silu(x):
    return jax.nn.silu(x)
def _sigmoid(x):
    return jax.nn.sigmoid(x)
def _layernorm(x, axis=-1, eps=1e-5):
    m = jnp.mean(x, axis=axis, keepdims=True)
    v = jnp.var(x, axis=axis, keepdims=True)
    return (x - m) / jnp.sqrt(v + eps)
def _scatter_add(tgt, idx, src, axis=0):
    return tgt.at[idx].add(src)
def _segment_sum(src, seg, n):
    return jax.ops.segment_sum(src, seg, n)
class _Rng:
    def __init__(self, key):
        self._k = key
    def _next(self):
        self._k, sub = jax.random.split(self._k)
        return sub
    def normal(self, shape):
        return jax.random.normal(self._next(), shape, dtype=jnp.bfloat16)
    def randint(self, lo, hi, shape):
        return jax.random.randint(self._next(), shape, lo, hi, dtype=jnp.int32)
    def uniform(self, shape, lo=0.0, hi=1.0):
        return jax.random.uniform(self._next(), shape, jnp.bfloat16, lo, hi)
    def permutation(self, n):
        return jax.random.permutation(self._next(), n)


kernel_name = 'recurrent_scan__sliding_block_cached__dense_activation_gelu__decode'

def setup_inputs():
    _rng = _Rng(jax.random.key(int.from_bytes(__import__("os").urandom(4), "little")))
    _w = (lambda a: (lambda t: t.astype(jnp.bfloat16) if jnp.issubdtype(t.dtype, jnp.floating) else t)(jnp.asarray(a)))
    def _A_setup():
        B, Sq, D = 2, 1, 576
        Hq, Hkv, Sk, Dh = 32, 16, 32768, 128
        assert Hq % Hkv == 0, (Hq, Hkv)
        return {
            "x": _w((lambda *s: _rng.normal(s) * 0.05)(B, Sq, D)),
            "k_cache": _w((lambda *s: _rng.normal(s) * 0.05)(B, Hkv, Sk, Dh)),
            "v_cache": _w((lambda *s: _rng.normal(s) * 0.05)(B, Hkv, Sk, Dh)),
            "wq": _w((lambda *s: _rng.normal(s) * 0.05)(D, Hq * Dh) * (D ** -0.5)),
            "wo": _w((lambda *s: _rng.normal(s) * 0.05)(Hq * Dh, D) * ((Hq * Dh) ** -0.5)),
        }
    _A_in = _A_setup()

    def _B_setup():
        B, S, D, F = 2, 1, 576, 4608
        return {
            "x": _w((lambda *s: _rng.normal(s) * 0.05)(B, S, D)),
            "w1": _w((lambda *s: _rng.normal(s) * 0.05)(D, F) * (D ** -0.5)),
            "b1": _w((lambda *s: _rng.normal(s) * 0.05)(F) * 0.01),
            "w2": _w((lambda *s: _rng.normal(s) * 0.05)(F, D) * (F ** -0.5)),
            "b2": _w((lambda *s: _rng.normal(s) * 0.05)(D) * 0.01),
        }
    _B_in = _B_setup()

    return {
        "A_x": _A_in["x"],
        "A_k_cache": _A_in["k_cache"],
        "A_v_cache": _A_in["v_cache"],
        "A_wq": _A_in["wq"],
        "A_wo": _A_in["wo"],
        "B_x": _B_in["x"],
        "B_w1": _B_in["w1"],
        "B_b1": _B_in["b1"],
        "B_w2": _B_in["w2"],
        "B_b2": _B_in["b2"],
    }

def reference(A_x, A_k_cache, A_v_cache, A_wq, A_wo, B_x, B_w1, B_b1, B_w2, B_b2):
    def _A_ref(x, k_cache, v_cache, wq, wo):
        B, Sq, D = x.shape
        Hq, Dh = 32, 128
        Hkv, Sk = k_cache.shape[1], k_cache.shape[2]
        W = min(4096, max(256, Sk // 4))
        rep = Hq // Hkv
        q = (lambda x, *d: x.transpose(*d))((x @ wq).reshape(B, Sq, Hq, Dh), 0, 2, 1, 3)
        k = jnp.repeat(k_cache[:, :, Sk - W:, :], rep, axis=1)
        v = jnp.repeat(v_cache[:, :, Sk - W:, :], rep, axis=1)
        scores = jnp.einsum("bhqd,bhkd->bhqk", q, k) * (Dh ** -0.5)
        p = _softmax(scores, axis=-1)
        o = jnp.einsum("bhqk,bhkd->bhqd", p, v)
        return (lambda x, *d: x.transpose(*d))(o, 0, 2, 1, 3).reshape(B, Sq, Hq * Dh) @ wo

    def _B_ref(x, w1, b1, w2, b2):
        h = jnp.einsum("bsd,df->bsf", x, w1) + b1
        h = _gelu(h)
        return jnp.einsum("bsf,fd->bsd", h, w2) + b2

    x = A_x
    xn = _layernorm(x, axis=-1)
    s = _A_ref(xn, A_k_cache, A_v_cache, A_wq, A_wo)
    g = _silu(_B_ref(xn, B_w1, B_b1, B_w2, B_b2))
    return x + s * g
```

```python
import jax
import jax.numpy as jnp
from jax import lax
from jax.experimental import pallas as pl
from jax.experimental.pallas import tpu as pltpu

_HQ, _DH = 32, 128
_ROWS = 8
_DEPTH = 4
_WCHUNK = 512
_NT = (((1,), (1,)), ((), ()))


def _kernel(x_h, k_h, v_h, wq_h, wo_h, w1_h, b1_h, w2_h, b2_h, o_ref,
            x_v, b1_v, b2_v, wq_v, w1_v, w2_v, wo_v, kv_v, sems, small_sems):
    f32, bf16 = jnp.float32, jnp.bfloat16
    nb, d = x_h.shape
    hkv, sk = k_h.shape[1], k_h.shape[2]
    win = kv_v.shape[2]
    ff = w1_h.shape[1]

    small = [pltpu.make_async_copy(s, t, small_sems.at[i])
             for i, (s, t) in enumerate(((x_h, x_v), (b1_h, b1_v), (b2_h, b2_v)))]
    queue = []

    def add(src, dst):
        queue.append(pltpu.make_async_copy(src, dst, sems.at[len(queue)]))
        return len(queue) - 1

    def add_cols(src, dst):
        return [(add(src.at[:, pl.ds(o, _WCHUNK)], dst.at[:, pl.ds(o, _WCHUNK)]), o)
                for o in range(0, src.shape[1], _WCHUNK)]

    wq_ids = add_cols(wq_h, wq_v)
    w1_ids = add_cols(w1_h, w1_v)
    w2_ids = add_cols(w2_h, w2_v)
    kv_ids = [[add(src.at[b, h, pl.ds(sk - win, win), :], kv_v.at[h, 2 * j + b])
               for j, src in enumerate((k_h, v_h)) for b in range(nb)] for h in range(hkv)]
    wo_ids = add_cols(wo_h, wo_v)

    def start(j):
        if j < len(queue):
            queue[j].start(priority=j % 2)

    def wait(j):
        queue[j].wait()
        start(j + _DEPTH)

    start(0)
    for c in small:
        c.start()
    for j in range(1, _DEPTH):
        start(j)
    for c in small:
        c.wait()

    row = lax.broadcasted_iota(jnp.int32, (_ROWS, 1), 0)
    batch0 = (row % 2) == 0
    head0 = (row % 4) < 2

    xf = x_v[...].astype(f32)
    x8 = jnp.where(batch0, xf[0:1], xf[1:2])
    xc = x8 - jnp.mean(x8, axis=-1, keepdims=True)
    var = jnp.mean(xc * xc, axis=-1, keepdims=True)
    xn = (xc / jnp.sqrt(var + 1e-5)).astype(bf16)

    qs = []
    for j, o in wq_ids:
        wait(j)
        qq = jnp.dot(xn, wq_v[:, o:o + _WCHUNK], preferred_element_type=f32)
        for t in range(0, _WCHUNK, 2 * _DH):
            qs.append(jnp.where(head0, qq[:, t:t + _DH], qq[:, t + _DH:t + 2 * _DH]).astype(bf16))

    b1 = b1_v[...].astype(f32).reshape(1, ff)
    hs = []
    for j, o in w1_ids:
        wait(j)
        hh = jnp.dot(xn, w1_v[:, o:o + _WCHUNK], preferred_element_type=f32) + b1[:, o:o + _WCHUNK]
        hs.append(jax.nn.gelu(hh, approximate=True).astype(bf16))
    g = jnp.zeros((_ROWS, d), f32)
    for (j, o), hh in zip(w2_ids, hs):
        wait(j)
        g = g + lax.dot_general(hh, w2_v[:, o:o + _WCHUNK], _NT, preferred_element_type=f32)
    g = g + b2_v[...].astype(f32).reshape(1, d)
    g = g * jax.nn.sigmoid(g)

    outs = []
    for h in range(hkv):
        ids = kv_ids[h]
        wait(ids[0])
        s0 = lax.dot_general(qs[h], kv_v[h, 0], _NT, preferred_element_type=f32)
        wait(ids[1])
        s1 = lax.dot_general(qs[h], kv_v[h, 1], _NT, preferred_element_type=f32)
        s = jnp.where(batch0, s0, s1) * (_DH ** -0.5)
        p = jnp.exp(s - jnp.max(s, axis=-1, keepdims=True))
        l = jnp.sum(p, axis=-1, keepdims=True)
        pb = p.astype(bf16)
        wait(ids[2])
        o0 = jnp.dot(pb, kv_v[h, 2], preferred_element_type=f32)
        wait(ids[3])
        o1 = jnp.dot(pb, kv_v[h, 3], preferred_element_type=f32)
        oo = jnp.where(batch0, o0, o1) / l
        outs.append(jnp.where(head0, oo, 0.0).astype(bf16))
        outs.append(jnp.where(head0, 0.0, oo).astype(bf16))

    acc = jnp.zeros((_ROWS, d), f32)
    for j, o in wo_ids:
        wait(j)
        lhs = jnp.concatenate(outs[o // _DH:(o + _WCHUNK) // _DH], axis=1)
        acc = acc + lax.dot_general(lhs, wo_v[:, o:o + _WCHUNK], _NT, preferred_element_type=f32)
    o_ref[...] = (xf + (acc[0:2] + acc[2:4]) * g[0:2]).astype(o_ref.dtype)


@jax.jit
def pallas_recurrent_scan__sliding_block_cached__dense_activation_gelu__decode_kernel(
    A_x: jax.Array,
    A_k_cache: jax.Array,
    A_v_cache: jax.Array,
    A_wq: jax.Array,
    A_wo: jax.Array,
    B_x: jax.Array,
    B_w1: jax.Array,
    B_b1: jax.Array,
    B_w2: jax.Array,
    B_b2: jax.Array,
):
    del B_x
    nb, sq, d = A_x.shape
    hkv, sk = A_k_cache.shape[1], A_k_cache.shape[2]
    ff = B_w1.shape[1]
    win = min(4096, max(256, sk // 4))
    assert (nb, sq) == (2, 1) and _HQ == 2 * hkv
    ncopies = 2 * (_HQ * _DH // _WCHUNK) + 2 * (ff // _WCHUNK) + 2 * nb * hkv
    out = pl.pallas_call(
        _kernel,
        out_shape=jax.ShapeDtypeStruct((nb, d), A_x.dtype),
        in_specs=[pl.BlockSpec(memory_space=pl.ANY)] * 9,
        scratch_shapes=[
            pltpu.VMEM((nb, d), A_x.dtype),
            pltpu.VMEM((ff,), B_b1.dtype),
            pltpu.VMEM((d,), B_b2.dtype),
            pltpu.VMEM((d, _HQ * _DH), A_wq.dtype),
            pltpu.VMEM((d, ff), B_w1.dtype),
            pltpu.VMEM((d, ff), B_w2.dtype),
            pltpu.VMEM((d, _HQ * _DH), A_wo.dtype),
            pltpu.VMEM((hkv, 2 * nb, win, _DH), A_k_cache.dtype),
            pltpu.SemaphoreType.DMA((ncopies,)),
            pltpu.SemaphoreType.DMA((3,)),
        ],
        compiler_params=pltpu.CompilerParams(vmem_limit_bytes=110 * 1024 * 1024),
    )(A_x.reshape(nb, d), A_k_cache, A_v_cache, A_wq, A_wo.T, B_w1, B_b1, B_w2.T, B_b2)
    return out.reshape(nb, sq, d)
```

```python
import jax
import jax.numpy as jnp
from jax import lax
from jax.experimental import pallas as pl
from jax.experimental.pallas import tpu as pltpu

_HQ, _DH = 32, 128
_ROWS = 8
_NSEM = 3
_COLS = 512
_KV_ROWS = 64
_KV_UNROLL = 8
_WO_PARTS = (2048, 1024, 512, 384, 128)
_NT = (((1,), (1,)), ((), ()))


def _kernel(x_h, k_h, v_h, wq_h, wo_h, w1_h, b1_h, w2_h, b2_h, o_ref,
            x_v, b1_v, b2_v, kv_v, q_v, a_v, h_v, g_v, acc_v, front_v, sems, *wo_v):
    f32, bf16 = jnp.float32, jnp.bfloat16
    d = x_h.shape[1]
    hkv, sk = k_h.shape[1], k_h.shape[2]
    win = kv_v.shape[2]
    nq, nf = wq_h.shape[1] // _COLS, w1_h.shape[1] // _COLS
    nfront = nq + 2 * nf

    def sem(g):
        return sems.at[g % _NSEM if isinstance(g, int) else lax.rem(g, _NSEM)]

    def wait(dst, g):
        pltpu.make_async_copy(dst, dst, sem(g)).wait()

    def issue_cols(src, off, dst, g):
        n = dst.shape[1]
        cols = [(o, min(_COLS, n - o)) for o in range(0, n, _COLS)]
        rep = 4 // len(cols)

        def body(r, carry):
            for u in range(rep):
                rows = pl.ds(pl.multiple_of((r * rep + u) * 16, 16), 16)
                for t, (o, w) in enumerate(cols):
                    pltpu.make_async_copy(src.at[rows, pl.ds(off + o, w)], dst.at[rows, pl.ds(o, w)],
                                          sem(g)).start(priority=(u * len(cols) + t) // 2 % 2)
            return carry

        lax.fori_loop(0, d // (16 * rep), body, 0)

    def issue_kv(h, half):
        def body(c, carry):
            base = pl.multiple_of(half * (win // 2) + c * _KV_ROWS * _KV_UNROLL, 16)
            for u in range(_KV_UNROLL):
                r = base + u * _KV_ROWS
                for j, src in enumerate((k_h, v_h)):
                    for b in range(2):
                        pltpu.make_async_copy(src.at[b, h, pl.ds(sk - win + r, _KV_ROWS), :],
                                              kv_v.at[h, 2 * j + b, pl.ds(r, _KV_ROWS)],
                                              sem(nfront + h)).start(priority=j)
            return carry

        lax.fori_loop(0, win // 2 // (_KV_ROWS * _KV_UNROLL), body, 0)

    front = [(w, j * _COLS) for w, n in ((wq_h, nq), (w1_h, nf), (w2_h, nf)) for j in range(n)]

    def issue_front(g):
        if g < nfront:
            issue_cols(*front[g], front_v.at[g], g)
        else:
            issue_kv(0, g - nfront)

    def next_front(g):
        issue_front(g + 2)
        wait(front_v.at[g], g)
        return front_v[g]

    small = [pltpu.make_async_copy(s, t, sem(2)) for s, t in ((x_h, x_v), (b1_h, b1_v), (b2_h, b2_v))]
    for c in small:
        c.start()
    issue_front(0)
    issue_front(1)
    for c in small:
        c.wait()

    row = lax.broadcasted_iota(jnp.int32, (_ROWS, 1), 0)
    batch0 = (row % 2) == 0
    head0 = (row % 4) < 2

    xf = x_v[...].astype(f32)
    x8 = jnp.where(batch0, xf[0:1], xf[1:2])
    xc = x8 - jnp.mean(x8, axis=-1, keepdims=True)
    var = jnp.mean(xc * xc, axis=-1, keepdims=True)
    xn = (xc / jnp.sqrt(var + 1e-5)).astype(bf16)

    for j in range(nq):
        qq = jnp.dot(xn, next_front(j), preferred_element_type=f32)
        for t in range(0, _COLS, 2 * _DH):
            q_v[(j * _COLS + t) // (2 * _DH)] = jnp.where(head0, qq[:, t:t + _DH], qq[:, t + _DH:t + 2 * _DH])

    b1 = b1_v[...].astype(f32).reshape(1, nf * _COLS)
    for j in range(nf):
        hh = jnp.dot(xn, next_front(nq + j), preferred_element_type=f32) + b1[:, j * _COLS:(j + 1) * _COLS]
        h_v[j] = jax.nn.gelu(hh, approximate=True)
    g_v[...] = jnp.broadcast_to(b2_v[...].astype(f32).reshape(1, d), (_ROWS, d))
    for j in range(nf):
        w2t = next_front(nq + nf + j)
        g_v[...] += lax.dot_general(h_v[j].astype(bf16), w2t, _NT, preferred_element_type=f32)
    gate = g_v[...]
    g_v[...] = gate * jax.nn.sigmoid(gate)

    def attend(h, issue_more):
        wait(kv_v.at[h], nfront + h)
        q = q_v[h].astype(bf16)
        s0 = lax.dot_general(q, kv_v[h, 0], _NT, preferred_element_type=f32)
        s1 = lax.dot_general(q, kv_v[h, 1], _NT, preferred_element_type=f32)
        s = jnp.where(batch0, s0, s1) * (_DH ** -0.5)
        p = jnp.exp(s - jnp.max(s, axis=-1, keepdims=True))
        l = jnp.sum(p, axis=-1, keepdims=True)
        pb = p.astype(bf16)
        issue_more()
        o0 = jnp.dot(pb, kv_v[h, 2], preferred_element_type=f32)
        o1 = jnp.dot(pb, kv_v[h, 3], preferred_element_type=f32)
        a_v[h] = jnp.where(batch0, o0, o1) / l

    def head(h, carry):
        issue_kv(h + 1, 0)
        attend(h, lambda: issue_kv(h + 1, 1))
        return carry

    lax.fori_loop(0, hkv - 1, head, 0)

    offs = [sum(_WO_PARTS[:j]) for j in range(len(_WO_PARTS))]

    def issue_wo(j):
        if j < len(wo_v):
            issue_cols(wo_h, offs[j], wo_v[j], nfront + hkv + j)

    issue_wo(0)
    attend(hkv - 1, lambda: issue_wo(1))
    acc_v[...] = jnp.zeros((_ROWS, d), f32)
    for j, (o, n) in enumerate(zip(offs, _WO_PARTS)):
        issue_wo(j + 2)
        wait(wo_v[j], nfront + hkv + j)
        lhs = [jnp.where(head0 == (t % 2 == 0), a_v[t // 2], 0.0).astype(bf16)
               for t in range(o // _DH, (o + n) // _DH)]
        acc_v[...] += lax.dot_general(jnp.concatenate(lhs, axis=1), wo_v[j][...], _NT,
                                      preferred_element_type=f32)
    acc = acc_v[...]
    o_ref[...] = (xf + (acc[0:2] + acc[2:4]) * g_v[0:2]).astype(o_ref.dtype)


@jax.jit
def pallas_recurrent_scan__sliding_block_cached__dense_activation_gelu__decode_kernel(
    A_x: jax.Array,
    A_k_cache: jax.Array,
    A_v_cache: jax.Array,
    A_wq: jax.Array,
    A_wo: jax.Array,
    B_x: jax.Array,
    B_w1: jax.Array,
    B_b1: jax.Array,
    B_w2: jax.Array,
    B_b2: jax.Array,
):
    del B_x
    nb, sq, d = A_x.shape
    hkv, sk = A_k_cache.shape[1], A_k_cache.shape[2]
    ff = B_w1.shape[1]
    win = min(4096, max(256, sk // 4))
    assert (nb, sq) == (2, 1) and _HQ == 2 * hkv and sum(_WO_PARTS) == _HQ * _DH
    assert ff % _COLS == 0 and d % 64 == 0 and win % (2 * _KV_ROWS * _KV_UNROLL) == 0
    f32, wdt = jnp.float32, A_wq.dtype
    out = pl.pallas_call(
        _kernel,
        out_shape=jax.ShapeDtypeStruct((nb, d), A_x.dtype),
        in_specs=[pl.BlockSpec(memory_space=pl.ANY)] * 9,
        scratch_shapes=[
            pltpu.VMEM((nb, d), A_x.dtype),
            pltpu.VMEM((ff,), B_b1.dtype),
            pltpu.VMEM((d,), B_b2.dtype),
            pltpu.VMEM((hkv, 2 * nb, win, _DH), A_k_cache.dtype),
            pltpu.VMEM((hkv, _ROWS, _DH), f32),
            pltpu.VMEM((hkv, _ROWS, _DH), f32),
            pltpu.VMEM((ff // _COLS, _ROWS, _COLS), f32),
            pltpu.VMEM((_ROWS, d), f32),
            pltpu.VMEM((_ROWS, d), f32),
            pltpu.VMEM(((_HQ * _DH + 2 * ff) // _COLS, d, _COLS), wdt),
            pltpu.SemaphoreType.DMA((_NSEM,)),
        ] + [pltpu.VMEM((d, n), wdt) for n in _WO_PARTS],
        compiler_params=pltpu.CompilerParams(vmem_limit_bytes=110 * 1024 * 1024),
    )(A_x.reshape(nb, d), A_k_cache, A_v_cache, A_wq, A_wo.T, B_w1, B_b1, B_w2.T, B_b2)
    return out.reshape(nb, sq, d)
```
